```python
import os as _os
_os.environ.setdefault('JAX_PLATFORMS', 'cpu')
import jax
import jax.numpy as jnp

def _softmax(x, axis=-1):
    return jax.nn.softmax(x, axis=axis)

def _gelu(x):
    return jax.nn.gelu(x, approximate=True)

def _silu(x):
    return jax.nn.silu(x)

def _sigmoid(x):
    return jax.nn.sigmoid(x)

def _layernorm(x, axis=-1, eps=1e-05):
    m = jnp.mean(x, axis=axis, keepdims=True)
    v = jnp.var(x, axis=axis, keepdims=True)
    return (x - m) / jnp.sqrt(v + eps)

def _scatter_add(tgt, idx, src, axis=0):
    return tgt.at[idx].add(src)

def _segment_sum(src, seg, n):
    return jax.ops.segment_sum(src, seg, n)

class _Rng:

    def __init__(self, key):
        self._k = key

    def _next(self):
        self._k, sub = jax.random.split(self._k)
        return sub

    def normal(self, shape):
        return jax.random.normal(self._next(), shape, dtype=jnp.bfloat16)

    def randint(self, lo, hi, shape):
        return jax.random.randint(self._next(), shape, lo, hi, dtype=jnp.int32)

    def uniform(self, shape, lo=0.0, hi=1.0):
        return jax.random.uniform(self._next(), shape, jnp.bfloat16, lo, hi)

    def permutation(self, n):
        return jax.random.permutation(self._next(), n)
kernel_name = 'gated_mix__sliding_block__memory_aug_recurrent_mem_tr__prompt'

def setup_inputs():
    _rng = _Rng(jax.random.key(int.from_bytes(__import__("os").urandom(4), "little")))
    _w = lambda a: (lambda t: t.astype(jnp.bfloat16) if jnp.issubdtype(t.dtype, jnp.floating) else t)(jnp.asarray(a))

    def _A_setup():
        B, S, D = (1, 2048, 448)
        return {'x': _w((lambda *s: _rng.normal(s) * 0.05)(B, S, D)), 'wqkv': _w((lambda *s: _rng.normal(s) * 0.8)(D, 3 * D)), 'wo': _w((lambda *s: _rng.normal(s) * 0.05)(D, D))}
    _A_in = _A_setup()

    def _B_setup():
        B, S, Dm = (1, 2048, 448)
        H, Dh = (16, 256)
        M, seg = (8, 32)
        seg = min(seg, S)
        S = S // seg * seg
        return {'x': _w((lambda *s: _rng.normal(s) * 0.05)(B, S, Dm)), 'mem0': _w((lambda *s: _rng.normal(s) * 0.8)(B, M, Dm)), 'Wq': _w((lambda *s: _rng.normal(s) * 3.2)(Dm, H, Dh) * Dm ** (-0.5)), 'Wk': _w((lambda *s: _rng.normal(s) * 3.2)(Dm, H, Dh) * Dm ** (-0.5)), 'Wv': _w((lambda *s: _rng.normal(s) * 0.8)(Dm, H, Dh) * Dm ** (-0.5)), 'Wo': _w((lambda *s: _rng.normal(s) * 0.8)(H, Dh, Dm) * (H * Dh) ** (-0.5)), 'seg_len': seg}
    _B_in = _B_setup()
    return {'A_x': _A_in['x'], 'A_wqkv': _A_in['wqkv'], 'A_wo': _A_in['wo'], 'B_x': _B_in['x'], 'B_mem0': _B_in['mem0'], 'B_Wq': _B_in['Wq'], 'B_Wk': _B_in['Wk'], 'B_Wv': _B_in['Wv'], 'B_Wo': _B_in['Wo'], 'B_seg_len': _B_in['seg_len'], 'gate_w': _w((lambda *s: _rng.normal(s) * 0.05)(448) * 16.0)}

def reference(A_x, A_wqkv, A_wo, B_x, B_mem0, B_Wq, B_Wk, B_Wv, B_Wo, B_seg_len, gate_w):

    def _A_ref(x, wqkv, wo):
        B, S, D = x.shape
        H = 16
        Dh = D // H
        W = 256
        qkv = (lambda x, *d: x.transpose(*d))((x @ wqkv).reshape(B, S, 3, H, Dh), 2, 0, 3, 1, 4)
        q, k, v = (qkv[0], qkv[1], qkv[2])
        scores = jnp.einsum('bhqd,bhkd->bhqk', q, k) * Dh ** (-0.5)
        idx = jnp.arange(S)
        mask = (idx[:, None] - idx[None, :] >= 0) & (idx[:, None] - idx[None, :] < W)
        scores = jnp.where(mask[None, None], scores, -1000000000.0)
        p = _softmax(scores, axis=-1)
        o = jnp.einsum('bhqk,bhkd->bhqd', p, v)
        return (lambda x, *d: x.transpose(*d))(o, 0, 2, 1, 3).reshape(B, S, D) @ wo

    def _B_ref(x, mem0, Wq, Wk, Wv, Wo, seg_len):
        B, S, Dm = x.shape
        H, Dh = (Wq.shape[1], Wq.shape[2])
        M = mem0.shape[1]
        scale = Dh ** (-0.5)
        n_seg = S // seg_len
        L = M + seg_len
        idx = jnp.arange(L)
        mask = (idx[:, None] < M) | (idx[:, None] >= idx[None, :])
        mem = mem0
        outs = []
        for s in range(n_seg):
            xs = x[:, s * seg_len:(s + 1) * seg_len, :].copy()
            h = jnp.concatenate([mem, xs], axis=1)
            q = jnp.einsum('btd,dhe->bhte', h, Wq)
            k = jnp.einsum('btd,dhe->bhte', h, Wk)
            v = jnp.einsum('btd,dhe->bhte', h, Wv)
            scores = jnp.einsum('bhqe,bhke->bhqk', q, k) * scale
            scores = jnp.where(mask[None, None], scores, -1000000000.0)
            p = _softmax(scores, axis=-1)
            o = jnp.einsum('bhqk,bhke->bhqe', p, v)
            o = jnp.einsum('bhte,hed->btd', o, Wo)
            mem = o[:, :M, :].copy()
            outs.append(o[:, M:, :])
        return jnp.concatenate(outs, axis=1)
    x = A_x
    g = _sigmoid((x * gate_w).sum(-1, keepdims=True))
    a = _A_ref(x, A_wqkv, A_wo)
    b = _B_ref(x, B_mem0, B_Wq, B_Wk, B_Wv, B_Wo, B_seg_len)
    return g * a + (1 - g) * b
```

```python
import functools
import os
import jax
import jax.numpy as jnp
from jax import lax
from jax.experimental import pallas as pl
from jax.experimental.pallas import tpu as pltpu

bf16, f32, u32 = jnp.bfloat16, jnp.float32, jnp.uint32

S, D = 2048, 448
AH, ADH, AW = 16, 28, 256
APD = 32
AN = AH * APD
H, DH, M, SEG = 16, 256, 8, 32
HW = 3 * DH
NQKV = H * HW
LOG2E = 1.4426950408889634
B_QSCALE = (DH ** -0.5) * LOG2E
A_QSCALE = (ADH ** -0.5) * LOG2E
NEG = -1e30
MASKVAL = -1e9
NSUPER = S // (2 * SEG)
LS, LV, LO = [int(a) for a in os.environ.get("LAGS", "1,3,4").split(",")]


def _relayout_w(w_ref, t_ref, wp_ref, part):
    def cp(j, _):
        r0 = pl.multiple_of(j * 128, 128)
        q0 = pl.multiple_of(j * 64, 64)
        for c in range(2):
            t_ref[c, pl.ds(q0, 64), :] = pltpu.bitcast(w_ref[pl.ds(r0, 128), c * 128:(c + 1) * 128], u32)
        return 0
    lax.fori_loop(0, 56, cp, 0)

    def body(g, _):
        r0 = pl.multiple_of(g * 128, 128)
        o0 = pl.multiple_of(g * 8, 8)
        for c in range(2):
            for i in range(8):
                a = t_ref[c, pl.ds(r0 + i, 8, stride=16), :]
                b = t_ref[c, pl.ds(r0 + 8 + i, 8, stride=16), :]
                x = (a & u32(0xFFFF)) | (b << 16)
                y = (a >> 16) | (b & u32(0xFFFF0000))
                ca = (2 * i) * HW + part * DH + c * 128
                cb = (2 * i + 1) * HW + part * DH + c * 128
                wp_ref[pl.ds(o0, 8), ca:ca + 128] = x
                wp_ref[pl.ds(o0, 8), cb:cb + 128] = y
        return 0
    lax.fori_loop(0, 28, body, 0)


def _perm_t(src0, w0, wl):
    n = lax.broadcasted_iota(jnp.int32, (128, wl), 0)
    s = lax.broadcasted_iota(jnp.int32, (128, wl), 1)
    tgt = src0 - w0 + ADH * (n >> 5) + (n & 31)
    hit = (s == tgt) & ((n & 31) < ADH)
    return jnp.where(hit, 1.0, 0.0).astype(bf16)


def _perm(src0, w0, wl):
    s = lax.broadcasted_iota(jnp.int32, (wl, 128), 0)
    n = lax.broadcasted_iota(jnp.int32, (wl, 128), 1)
    tgt = src0 - w0 + ADH * (n >> 5) + (n & 31)
    hit = (s == tgt) & ((n & 31) < ADH)
    return jnp.where(hit, 1.0, 0.0).astype(bf16)


def _window(src0, total):
    w0 = (src0 // 128) * 128
    w1 = min(-(-(src0 + 4 * ADH) // 128) * 128, total)
    return w0, w1 - w0


_NT = (((1,), (1,)), ((), ()))


def _kernel(xaT_ref, wqkv_ref, woa_ref, mem0_ref, wq_ref, wk_ref, wv_ref, woT_ref, gate_ref,
            out_ref,
            t_ref, wp_ref, wop_ref, xb_ref, ringA, ringB, oA, oB, bst_ref,
            wT_ref, wkp_ref, woTp_ref, qT_ref, kA_ref, vT_ref, g_ref, pT_ref, r_ref, oT_ref, outT_ref):
    for g in range(4):
        for part, row0 in ((0, 0), (2, AN)):
            src0 = part * D + 4 * ADH * g
            w0, wl = _window(src0, 3 * D)
            y = lax.dot_general(_perm_t(src0, w0, wl), wqkv_ref[:, w0:w0 + wl], _NT, preferred_element_type=f32)
            wT_ref[row0 + 128 * g: row0 + 128 * (g + 1), :] = y.astype(bf16)
        src0 = D + 4 * ADH * g
        w0, wl = _window(src0, 3 * D)
        y = jnp.dot(wqkv_ref[:, w0:w0 + wl], _perm(src0, w0, wl), preferred_element_type=f32)
        wkp_ref[:, 128 * g:128 * (g + 1)] = y.astype(bf16)
        src0 = 4 * ADH * g
        w0, wl = _window(src0, D)
        y = jnp.dot(_perm_t(src0, w0, wl), woa_ref[w0:w0 + wl, :], preferred_element_type=f32)
        woTp_ref[:, 128 * g:128 * (g + 1)] = y.T.astype(bf16)
    wT_ref[2 * AN:2 * AN + 16, :] = jnp.broadcast_to(gate_ref[...].reshape(1, D), (16, D))

    lane = lax.broadcasted_iota(jnp.int32, (AW, AN), 1)
    kA_ref[0:AW, :] = jnp.where((lane & 31) == ADH, 1.0, 0.0).astype(bf16)
    vT_ref[:, 0:AW] = jnp.zeros((AN, AW), bf16)
    pT_ref[...] = jnp.zeros(pT_ref.shape, bf16)
    r_ref[...] = jnp.zeros(r_ref.shape, f32)
    oT_ref[...] = jnp.zeros(oT_ref.shape, bf16)
    bst_ref[...] = jnp.zeros(bst_ref.shape, f32)
    oA[...] = jnp.zeros(oA.shape, bf16)
    oB[...] = jnp.zeros(oB.shape, bf16)

    CH = 256
    def aproj(c, _):
        c0 = pl.multiple_of(c * CH, CH)
        xT = xaT_ref[:, pl.ds(c0, CH)]
        y = jnp.dot(wT_ref[...], xT, preferred_element_type=f32)
        row = lax.broadcasted_iota(jnp.int32, (AN, CH), 0)
        q = jnp.where((row & 31) == ADH, MASKVAL, y[0:AN] * A_QSCALE)
        qT_ref[:, pl.ds(c0, CH)] = q.astype(bf16)
        vT_ref[:, pl.ds(AW + c0, CH)] = y[AN:2 * AN].astype(bf16)
        g_ref[:, pl.ds(c0, CH)] = jax.nn.sigmoid(y[2 * AN:2 * AN + 8])
        xr = xT.T
        kA_ref[pl.ds(AW + c0, CH), :] = jnp.dot(xr, wkp_ref[...], preferred_element_type=f32).astype(bf16)
        xb_ref[pl.ds(c0, CH), :] = xr
        return 0
    lax.fori_loop(0, S // CH, aproj, 0)

    _relayout_w(wq_ref, t_ref, wp_ref, 0)
    _relayout_w(wk_ref, t_ref, wp_ref, 1)
    _relayout_w(wv_ref, t_ref, wp_ref, 2)

    def cpo(h, _):
        r0 = pl.multiple_of(h * D, 64)
        q0 = pl.multiple_of(h * 128, 128)
        wop_ref[pl.ds(q0, 128), :] = pltpu.bitcast(woT_ref[pl.ds(r0, D), :].T, u32)
        return 0
    lax.fori_loop(0, H, cpo, 0)

    ri = lax.broadcasted_iota(jnp.int32, (48, 48), 0)
    ci = lax.broadcasted_iota(jnp.int32, (48, 48), 1)
    allowed = (ci < 40) & ((ri >= 32) | (ci >= 32) | (ci <= ri))
    zpad = jnp.zeros((8, HW), f32)
    trow = lax.broadcasted_iota(jnp.int32, (128, AN), 0)
    tcol = lax.broadcasted_iota(jnp.int32, (128, AN), 1) & 127
    tri = trow <= tcol

    def proj_head(L, h):
        w = pltpu.bitcast(wp_ref[:, h * HW:(h + 1) * HW], bf16)
        y = jnp.dot(L, w, preferred_element_type=f32)
        return jnp.concatenate([y[:, :DH] * B_QSCALE, y[:, DH:]], axis=1)

    def a_scores(blk, g):
        b0 = pl.multiple_of(blk * 128, 128)
        qg = qT_ref[128 * g:128 * (g + 1), pl.ds(b0, 128)]
        ws = []
        for hh in range(4):
            parts = []
            if hh > 0:
                parts.append(jnp.zeros((32 * hh, 128), bf16))
            parts.append(qg[32 * hh:32 * (hh + 1)])
            if hh < 3:
                parts.append(jnp.zeros((96 - 32 * hh, 128), bf16))
            ws.append(jnp.concatenate(parts, axis=0))
        w = jnp.concatenate(ws, axis=1)
        kr = kA_ref[pl.ds(b0, 384), 128 * g:128 * (g + 1)]
        s = jnp.dot(kr, w, preferred_element_type=f32)
        sm = jnp.where(tri, s[256:384], s[0:128])
        s2 = s[128:256]
        m = jnp.maximum(jnp.max(sm, axis=0, keepdims=True), jnp.max(s2, axis=0, keepdims=True))
        em = jnp.exp2(sm - m)
        e2 = jnp.exp2(s2 - m)
        l = jnp.sum(em, axis=0, keepdims=True) + jnp.sum(e2, axis=0, keepdims=True)
        pT_ref[0:128, :] = jnp.where(tri, 0.0, em).astype(bf16)
        pT_ref[128:256, :] = e2.astype(bf16)
        pT_ref[256:384, :] = jnp.where(tri, em, 0.0).astype(bf16)
        r = pl.reciprocal(l, approx=True)
        r = r * (2.0 - l * r)
        r_ref[...] = jnp.broadcast_to(r, r_ref.shape)

    def a_pv(blk, g):
        b0 = pl.multiple_of(blk * 128, 128)
        for hh in range(4):
            h = 4 * g + hh
            v = vT_ref[32 * h:32 * (h + 1), pl.ds(b0, 384)]
            o = jnp.dot(v, pT_ref[:, 128 * hh:128 * (hh + 1)], preferred_element_type=f32)
            o = o * r_ref[0:1, 128 * hh:128 * (hh + 1)]
            oT_ref[32 * h:32 * (h + 1), :] = o.astype(bf16)

    def a_out():
        return jnp.dot(woTp_ref[...], oT_ref[...], preferred_element_type=f32)

    def combine(aT, slot):
        c0 = slot * 128
        gb = jnp.maximum(slot - 1, 0) * 128
        if not isinstance(slot, int):
            c0 = pl.multiple_of(c0, 128)
            gb = pl.multiple_of(gb, 128)
        else:
            gb = max(slot - 1, 0) * 128
        g = g_ref[0:1, pl.ds(gb, 128)]
        bT = bst_ref[...].T
        outT_ref[:, pl.ds(c0, 128)] = (g * aT + (1.0 - g) * bT).astype(bf16)

    def step(mem, xrows, rc, rc_base, n_targets, oc_targets, op, op_base, nrows, fill):
        L = jnp.concatenate([mem, xrows], axis=0)
        ys, es, os_ = {}, {}, {}
        acc = [None]

        def do_proj(h):
            y = proj_head(L, h)
            yb = y.astype(bf16)
            for (r0, n, ref, d0) in n_targets:
                ref[d0:d0 + n, h * HW:(h + 1) * HW] = yb[r0:r0 + n]
            ys[h] = jnp.concatenate([y[0:8], zpad], axis=0).astype(bf16)

        def do_scores(h):
            tok = rc[rc_base:rc_base + 32, h * HW:(h + 1) * HW]
            a = jnp.concatenate([tok, ys.pop(h)], axis=0)
            q = a[:, :DH]; k = a[:, DH:2 * DH]; v = a[:, 2 * DH:]
            s = lax.dot_general(q, k, _NT, preferred_element_type=f32)
            s = jnp.where(allowed, s, NEG)
            m = jnp.max(s, axis=1, keepdims=True)
            e = jnp.exp2(s - m)
            l = jnp.sum(e, axis=1, keepdims=True)
            r = pl.reciprocal(l, approx=True)
            r = r * (2.0 - l * r)
            es[h] = ((e * r).astype(bf16), v)

        def do_pv(h):
            p, v = es.pop(h)
            o = jnp.dot(p, v, preferred_element_type=f32).astype(bf16)
            for (r0, n, ref, d0) in oc_targets:
                ref[d0:d0 + n, h * DH:(h + 1) * DH] = o[r0:r0 + n]
            os_[h] = o[32:40]

        def do_oproj(h):
            lhs = jnp.concatenate([os_.pop(h), op[op_base + 8:op_base + nrows, h * DH:(h + 1) * DH]], axis=0)
            w = pltpu.bitcast(wop_ref[h * 128:(h + 1) * 128, :], bf16)
            y = jnp.dot(lhs, w, preferred_element_type=f32)
            acc[0] = y if acc[0] is None else acc[0] + y

        for t in range(H + LO + 1):
            for fn in fill.get(t, ()):
                fn()
            if t < H: do_proj(t)
            if 0 <= t - LS < H: do_scores(t - LS)
            if 0 <= t - LV < H: do_pv(t - LV)
            if 0 <= t - LO < H: do_oproj(t - LO)
        return acc[0]

    L0 = xb_ref[0:64, :]
    for h in range(H):
        ringA[:, h * HW:(h + 1) * HW] = proj_head(L0, h).astype(bf16)

    def superstep(j, mem, rc, rn, oc, op, bst_base, fills):
        nx = pl.multiple_of(jnp.minimum(j + 1, NSUPER - 1) * 64, 64)
        xn = xb_ref[pl.ds(nx, 64), :]
        y2 = step(mem, xn[0:24], rc, 0, [(8, 24, rn, 0)], [(0, 24, oc, 8), (24, 8, oc, 40)], op, 0, 32, fills[0])
        mem = y2[0:8].astype(bf16)
        bst_ref[bst_base:bst_base + 24, :] = y2[8:32]
        y2 = step(mem, xn[24:64], rc, 32, [(8, 40, rn, 24)], [(0, 32, oc, 48)], op, 32, 48, fills[1])
        mem = y2[0:8].astype(bf16)
        bst_ref[bst_base + 24:bst_base + 64, :] = y2[8:48]
        return mem

    FS = int(os.environ.get("FS", H))
    FV = int(os.environ.get("FV", 2))
    FO = int(os.environ.get("FO", H + 2))

    def body(i, mem):
        prev = jnp.maximum(i - 1, 0)
        aT = []
        f0 = {FV: [lambda: a_pv(prev, 3)], FS: [lambda: a_scores(i, 0)]}
        f1 = {FV: [lambda: a_pv(i, 0)], FS: [lambda: a_scores(i, 1)]}
        f0.setdefault(FO, []).append(lambda: aT.append(a_out()))
        mem = superstep(2 * i, mem, ringA, ringB, oA, oB, 64, (f0, f1))
        combine(aT[0], i)
        f2 = {FV: [lambda: a_pv(i, 1)], FS: [lambda: a_scores(i, 2)]}
        f3 = {FV: [lambda: a_pv(i, 2)], FS: [lambda: a_scores(i, 3)]}
        mem = superstep(2 * i + 1, mem, ringB, ringA, oB, oA, 0, (f2, f3))
        return mem

    lax.fori_loop(0, NSUPER // 2, body, mem0_ref[...])

    nb = S // 128
    a_pv(nb - 1, 3)
    aT = a_out()
    w = pltpu.bitcast(wop_ref[...], bf16)
    y2 = jnp.dot(oB[...], w, preferred_element_type=f32)
    bst_ref[64:88, :] = y2[8:32]
    bst_ref[88:128, :] = y2[40:80]
    combine(aT, nb)
    out_ref[...] = outT_ref[:, 128:]


@functools.partial(jax.jit, static_argnames=("B_seg_len",))
def pallas_gated_mix__sliding_block__memory_aug_recurrent_mem_tr__prompt_kernel(A_x, A_wqkv, A_wo, B_x, B_mem0, B_Wq, B_Wk, B_Wv, B_Wo, B_seg_len, gate_w):
    assert B_seg_len == SEG
    xaT = jnp.swapaxes(A_x, 1, 2).reshape(D, S)
    mem0 = B_mem0.reshape(M, D)
    wq = B_Wq.reshape(D * H, DH); wk = B_Wk.reshape(D * H, DH); wv = B_Wv.reshape(D * H, DH)
    woT = jnp.swapaxes(B_Wo, 1, 2).reshape(H * D, DH)
    outT = pl.pallas_call(
        _kernel,
        out_shape=jax.ShapeDtypeStruct((D, S), bf16),
        scratch_shapes=[
            pltpu.VMEM((2, 3584, 128), u32),
            pltpu.VMEM((224, NQKV), u32),
            pltpu.VMEM((H * 128, D), u32),
            pltpu.VMEM((S, D), bf16),
            pltpu.VMEM((64, NQKV), bf16), pltpu.VMEM((64, NQKV), bf16),
            pltpu.VMEM((80, H * DH), bf16), pltpu.VMEM((80, H * DH), bf16),
            pltpu.VMEM((128, D), f32),
            pltpu.VMEM((2 * AN + 16, D), bf16),
            pltpu.VMEM((D, AN), bf16),
            pltpu.VMEM((D, AN), bf16),
            pltpu.VMEM((AN, S), bf16),
            pltpu.VMEM((AW + S, AN), bf16),
            pltpu.VMEM((AN, AW + S), bf16),
            pltpu.VMEM((8, S), f32),
            pltpu.VMEM((384, AN), bf16),
            pltpu.VMEM((8, AN), f32),
            pltpu.VMEM((AN, 128), bf16),
            pltpu.VMEM((D, S + 128), bf16),
        ],
        compiler_params=pltpu.CompilerParams(vmem_limit_bytes=120 * 1024 * 1024),
    )(xaT, A_wqkv, A_wo, mem0, wq, wk, wv, woT, gate_w)
    return jnp.swapaxes(outT.reshape(1, D, S), 1, 2)
```

```python
import functools
import os
import jax
import jax.numpy as jnp
from jax import lax
from jax.experimental import pallas as pl
from jax.experimental.pallas import tpu as pltpu

bf16, f32, u32 = jnp.bfloat16, jnp.float32, jnp.uint32

S, D = 2048, 448
ADH, AW = 28, 256
APD = 32
AN = 16 * APD
H, DH, M, SEG = 16, 256, 8, 32
HW = 3 * DH
NQKV = H * HW
LOG2E = 1.4426950408889634
B_QSCALE = (DH ** -0.5) * LOG2E
A_QSCALE = (ADH ** -0.5) * LOG2E
NEG = -1e30
MASKVAL = -1e9
NSUPER = S // (2 * SEG)
NBLK = S // 128
NSTART0 = int(os.environ.get('NSTART0', '7'))
EARLYV = 1
NXLU = int(os.environ.get('NXLU', '4'))
RELAY = os.environ.get('RELAY', 'mem')
KLOOP = int(os.environ.get('KLOOP', '0'))
CH = 256


def _default_order():
    o = ["K0", "K1"]
    for t in range(16):
        if t + 2 < 16: o.append("K%d" % (t + 2))
        if t == 0: o.append("S0")
        if t + 1 < 16: o.append("S%d" % (t + 1))
        o.append("P%d" % t)
        if t == 1: o.append("c2")
        if t == 2: o.append("c3")
        if t >= 1: o.append("V%d" % (t - 1))
        if t >= 2: o.append("O%d" % (t - 2))
    o += os.environ.get("TAIL", "a0 a1 V15 O14 a2 a3 O15 d0 b0 b1").split()
    return o


ORDER = os.environ["ORDER"].split() if "ORDER" in os.environ else _default_order()

_NT = (((1,), (1,)), ((), ()))


def _perm_t(off, wl):
    n = lax.broadcasted_iota(jnp.int32, (128, wl), 0)
    s = lax.broadcasted_iota(jnp.int32, (128, wl), 1)
    hit = (s == off + ADH * (n >> 5) + (n & 31)) & ((n & 31) < ADH)
    return jnp.where(hit, 1.0, 0.0).astype(bf16)


def _perm(off, wl):
    s = lax.broadcasted_iota(jnp.int32, (wl, 128), 0)
    n = lax.broadcasted_iota(jnp.int32, (wl, 128), 1)
    hit = (s == off + ADH * (n >> 5) + (n & 31)) & ((n & 31) < ADH)
    return jnp.where(hit, 1.0, 0.0).astype(bf16)


def _wstart(src0, total):
    return min((src0 // 128) * 128, total - 256)


def _kernel(xaT_hbm, wqkv_hbm, woa_hbm, mem0_hbm, wq_hbm, wk_hbm, wv_hbm, woT_hbm, gate_hbm,
            out_hbm,
            sems, xaT_ref, wqkv_ref, woa_ref, mem0_ref, gate_ref, wr0, wr1, wr2, wr3,
            t_ref, wp_ref, wop_ref, xb_ref, ringE, ringOA, ringOB, oE, oOA, oOB, bst_ref,
            wT_ref, wkp_ref, woTp_ref, qT_ref, kA_ref, vT_ref, g_ref, pT_ref, oT_ref, outT_ref, aT_ref,
            pmt_ref, pmk_ref):
    def cp(src, dst, k):
        return pltpu.make_async_copy(src, dst, sems.at[k])

    c_wqkv, c_xa, c_woa = cp(wqkv_hbm, wqkv_ref, 0), cp(xaT_hbm, xaT_ref, 1), cp(woa_hbm, woa_ref, 2)
    c_gate, c_mem0 = cp(gate_hbm, gate_ref, 3), cp(mem0_hbm, mem0_ref, 4)
    c_wq, c_wk, c_wv, c_wo = cp(wq_hbm, wr0, 5), cp(wk_hbm, wr1, 6), cp(wv_hbm, wr2, 7), cp(woT_hbm, wr3, 8)
    for c in (c_wqkv, c_gate, c_xa, c_mem0, c_woa, c_wq, c_wk)[:NSTART0]:
        c.start()

    qwin = [(112 * g // 128) * 128 for g in range(4)]
    kwin = [((D + 112 * g) // 128) * 128 for g in range(4)]
    qwl = [min(256, 3 * D - (2 * D + w)) for w in qwin]
    kwl = [256, 256, 256, 128]
    for g in range(4):
        pmt_ref[g] = _perm_t(112 * g - qwin[g], 256)
        pmk_ref[g] = _perm(D + 112 * g - kwin[g], 256)
    lane = lax.broadcasted_iota(jnp.int32, (AW // 2, 128), 1)
    for g in range(4):
        kA_ref[g, 0:AW // 2, :] = jnp.where((lane & 31) == ADH, u32(0x3F803F80), u32(0))
    vT_ref[:, 0:AW] = jnp.zeros((AN, AW), bf16)
    pT_ref[...] = jnp.ones(pT_ref.shape, bf16)
    aT_ref[...] = jnp.zeros(aT_ref.shape, f32)
    oT_ref[...] = jnp.zeros(oT_ref.shape, u32)
    bst_ref[...] = jnp.zeros(bst_ref.shape, f32)
    oOB[...] = jnp.zeros(oOB.shape, bf16)

    c_wqkv.wait()
    for c in (c_wqkv, c_gate, c_xa, c_mem0, c_woa, c_wq, c_wk)[NSTART0:]:
        c.start()
    if EARLYV:
        c_wv.start()
        c_wo.start()
    for g in range(4):
        for base, row0 in ((0, 0), (2 * D, AN)):
            w0, wl = base + qwin[g], qwl[g]
            y = lax.dot_general(pmt_ref[g, :, 0:wl], wqkv_ref[:, w0:w0 + wl], _NT, preferred_element_type=f32)
            wT_ref[row0 + 128 * g: row0 + 128 * (g + 1), :] = y.astype(bf16)
        w0, wl = kwin[g], kwl[g]
        y = jnp.dot(wqkv_ref[:, w0:w0 + wl], pmk_ref[g, 0:wl, :], preferred_element_type=f32)
        wkp_ref[:, 128 * g:128 * (g + 1)] = y.astype(bf16)
    c_gate.wait()
    wT_ref[2 * AN:2 * AN + 16, :] = jnp.broadcast_to(gate_ref[...].reshape(1, D), (16, D))
    c_xa.wait()

    def relayout_unit(w_ref, part, g, slot):
        r0 = pl.multiple_of(g * 256, 256)
        o0 = pl.multiple_of(g * 8, 8)
        for c in range(2):
            t = pltpu.bitcast(w_ref[pl.ds(r0, 256), c * 128:(c + 1) * 128], u32)
            for dd in range(16):
                p0 = (dd % 2) * 64 + (dd // 2) * 8
                t_ref[slot, c, p0:p0 + 8, :] = t[dd * 8:(dd + 1) * 8]
        for c in range(2):
            for i in range(8):
                a = t_ref[slot, c, pl.ds(i, 8, stride=8), :]
                b = t_ref[slot, c, pl.ds(64 + i, 8, stride=8), :]
                x = (a & u32(0xFFFF)) | (b << 16)
                y = (a >> 16) | (b & u32(0xFFFF0000))
                ca = (2 * i) * HW + part * DH + c * 128
                cb = (2 * i + 1) * HW + part * DH + c * 128
                wp_ref[pl.ds(o0, 8), ca:ca + 128] = x
                wp_ref[pl.ds(o0, 8), cb:cb + 128] = y

    def aproj(c, extra):
        extra = list(extra)
        per = -(-len(extra) // 5)

        def run_extra():
            for _ in range(per):
                if extra:
                    extra.pop(0)()

        c0 = pl.multiple_of(c * CH, CH)
        xT = xaT_ref[:, pl.ds(c0, CH)]
        row = lax.broadcasted_iota(jnp.int32, (256, CH), 0)
        for p in range(2):
            y = jnp.dot(wT_ref[256 * p:256 * (p + 1), :], xT, preferred_element_type=f32)
            q = jnp.where((row & 31) == ADH, MASKVAL, y * A_QSCALE)
            qT_ref[256 * p:256 * (p + 1), pl.ds(c0, CH)] = q.astype(bf16)
            run_extra()
        y = jnp.dot(wT_ref[AN:AN + 256, :], xT, preferred_element_type=f32)
        vT_ref[0:256, pl.ds(AW + c0, CH)] = jnp.where((row & 31) == ADH, 1.0, y).astype(bf16)
        run_extra()
        y = jnp.dot(wT_ref[AN + 256:2 * AN + 16, :], xT, preferred_element_type=f32)
        vT_ref[256:512, pl.ds(AW + c0, CH)] = jnp.where((row & 31) == ADH, 1.0, y[0:256]).astype(bf16)
        g_ref[:, pl.ds(c0, CH)] = jax.nn.sigmoid(y[256:264])
        run_extra()
        xr = xT.T
        if not KLOOP:
            kk = jnp.dot(xr, wkp_ref[...], preferred_element_type=f32).astype(bf16)
            for g in range(4):
                kA_ref[g, pl.ds(pl.multiple_of((AW + c0) // 2, 64), CH // 2), :] = pltpu.bitcast(kk[:, 128 * g:128 * (g + 1)], u32)
        xb_ref[pl.ds(c0, CH), :] = xr
        run_extra()

    def k_proj(blk, g):
        r0 = pl.multiple_of(blk * 128, 128)
        kk = jnp.dot(xb_ref[pl.ds(r0, 128), :], wkp_ref[:, 128 * g:128 * (g + 1)], preferred_element_type=f32)
        kA_ref[g, pl.ds(pl.multiple_of((AW + r0) // 2, 64), 64), :] = pltpu.bitcast(kk.astype(bf16), u32)

    def aproj1(c, _):
        aproj(2 * c, [])
        aproj(2 * c + 1, [])
        return 0
    lax.fori_loop(0, 2, aproj1, 0)
    c_wq.wait()

    def aproj2(c, _, w_ref, part, c_first):
        ex = [functools.partial(relayout_unit, w_ref, part, c * 14 + u, u) for u in range(14)]
        aproj(c_first + c, ex)
        return 0
    lax.fori_loop(0, 2, functools.partial(aproj2, w_ref=wr0, part=0, c_first=4), 0)
    c_wk.wait()
    lax.fori_loop(0, 2, functools.partial(aproj2, w_ref=wr1, part=1, c_first=6), 0)

    c_wv.wait()
    c_woa.wait()
    c_mem0.wait()
    L0 = xb_ref[0:48, :]
    if KLOOP:
        for g in range(4):
            k_proj(0, g)

    def pro_qk(c, _):
        w0 = pl.multiple_of(jnp.minimum((112 * c // 128) * 128, D - 256), 64)
        n = lax.broadcasted_iota(jnp.int32, (128, 256), 0)
        s = lax.broadcasted_iota(jnp.int32, (128, 256), 1)
        hit = (s == 112 * c - w0 + ADH * (n >> 5) + (n & 31)) & ((n & 31) < ADH)
        y = jnp.dot(jnp.where(hit, 1.0, 0.0).astype(bf16), woa_ref[pl.ds(w0, 256), :], preferred_element_type=f32)
        woTp_ref[c] = pltpu.bitcast(y.T.astype(bf16), u32)
        for hh in range(4):
            c0 = pl.multiple_of((c * 4 + hh) * HW, 128)
            w = pltpu.bitcast(wp_ref[:, pl.ds(c0, 2 * DH)], bf16)
            y = jnp.dot(L0, w, preferred_element_type=f32)
            y = jnp.concatenate([y[:, :DH] * B_QSCALE, y[:, DH:]], axis=1)
            yb = y.astype(bf16)
            ringE[:, pl.ds(c0, 2 * DH)] = yb[0:32]
            ringOA[0:8, pl.ds(c0, 2 * DH)] = yb[32:40]
            for u in range(2 * hh, min(2 * hh + 2, 7)):
                relayout_unit(wr2, 2, c * 7 + u, u)
        return 0
    lax.fori_loop(0, 4, pro_qk, 0)
    c_wo.wait()

    def pro_v(c, _):
        for hh in range(4):
            h = c * 4 + hh
            c0 = pl.multiple_of(h * HW + 2 * DH, 128)
            w = pltpu.bitcast(wp_ref[:, pl.ds(c0, DH)], bf16)
            yb = jnp.dot(L0, w, preferred_element_type=f32).astype(bf16)
            ringE[:, pl.ds(c0, DH)] = yb[0:32]
            ringOA[0:8, pl.ds(c0, DH)] = yb[32:40]
            r0 = pl.multiple_of(h * D, 64)
            q0 = pl.multiple_of(h * 128, 128)
            wop_ref[pl.ds(q0, 128), :] = pltpu.bitcast(wr3[pl.ds(r0, D), :].T, u32)
        return 0
    lax.fori_loop(0, 4, pro_v, 0)

    ri = lax.broadcasted_iota(jnp.int32, (48, 48), 0)
    ci = lax.broadcasted_iota(jnp.int32, (48, 48), 1)
    allowed = (ci < 40) & ((ri >= 32) | (ci >= 32) | (ci <= ri))
    tri = lax.broadcasted_iota(jnp.int32, (128, 128), 0) <= lax.broadcasted_iota(jnp.int32, (128, 128), 1)

    def a_scores(blk, g, hh):
        b0 = pl.multiple_of(blk * 128, 128)
        h = 4 * g + hh
        parts = []
        if hh > 0:
            parts.append(jnp.zeros((32 * hh, 128), bf16))
        parts.append(qT_ref[32 * h:32 * (h + 1), pl.ds(b0, 128)])
        if hh < 3:
            parts.append(jnp.zeros((96 - 32 * hh, 128), bf16))
        w = jnp.concatenate(parts, axis=0)
        kr = pltpu.bitcast(kA_ref[g, pl.ds(pl.multiple_of(blk * 64, 64), 192), :], bf16)
        s = jnp.dot(kr, w, preferred_element_type=f32)
        sm = jnp.where(tri, s[256:384], s[0:128])
        s2 = s[128:256]
        m = jnp.max(jnp.maximum(sm, s2), axis=0, keepdims=True)
        em = jnp.exp2(sm - m)
        e2 = jnp.exp2(s2 - m)
        pT_ref[hh, 0:128, :] = jnp.where(tri, 0.0, em).astype(bf16)
        pT_ref[hh, 128:256, :] = e2.astype(bf16)
        pT_ref[hh, 256:384, :] = jnp.where(tri, em, 0.0).astype(bf16)

    def a_pv(blk, g, hh):
        b0 = pl.multiple_of(blk * 128, 128)
        h = 4 * g + hh
        v = vT_ref[32 * h:32 * (h + 1), pl.ds(b0, 384)]
        o = jnp.dot(v, pT_ref[hh], preferred_element_type=f32)
        l = o[ADH:ADH + 1, :]
        r = pl.reciprocal(l, approx=True)
        r = r * (2.0 - l * r)
        o = o * r
        oT_ref[lax.rem(blk, 2), 16 * h:16 * (h + 1), :] = pltpu.bitcast(o.astype(bf16), u32)

    def a_out(par, r0, n):
        lhs = pltpu.bitcast(jnp.concatenate([woTp_ref[g, r0 // 2:(r0 + n) // 2, :] for g in range(4)], axis=1), bf16)
        aT_ref[par, r0:r0 + n, :] = jnp.dot(lhs, pltpu.bitcast(oT_ref[par], bf16), preferred_element_type=f32)

    def combine(par, slot, gblk):
        c0 = pl.multiple_of(slot * 128, 128)
        gb = pl.multiple_of(gblk * 128, 128)
        g = g_ref[0:1, pl.ds(gb, 128)]
        bT = bst_ref[par].T
        outT_ref[:, pl.ds(c0, 128)] = (g * aT_ref[par] + (1.0 - g) * bT).astype(bf16)

    def out_copy(blk):
        c0 = pl.multiple_of(blk * 128, 128)
        return pltpu.make_async_copy(outT_ref.at[:, pl.ds(256 + c0, 128)], out_hbm.at[:, pl.ds(c0, 128)], sems.at[9])

    def step(mem, xrows, rc, n_targets, oc, op_pieces, fill):
        L = jnp.concatenate([mem, xrows], axis=0)
        yqk, yv, es, os_ = {}, {}, {}, {}
        acc = [None]

        def store_tok(yb, c0, w):
            for (r0, n, ref, d0) in n_targets:
                ref[d0:d0 + n, c0:c0 + w] = yb[r0:r0 + n]

        def do_pqk(h):
            c0 = h * HW
            w = pltpu.bitcast(wp_ref[:, c0:c0 + 2 * DH], bf16)
            y = jnp.dot(L, w, preferred_element_type=f32)
            y = jnp.concatenate([y[:, :DH] * B_QSCALE, y[:, DH:]], axis=1)
            store_tok(y.astype(bf16), c0, 2 * DH)
            yqk[h] = jnp.concatenate([y[0:8], jnp.zeros((8, 2 * DH), f32)], axis=0).astype(bf16)

        def do_pv(h):
            c0 = h * HW + 2 * DH
            w = pltpu.bitcast(wp_ref[:, c0:c0 + DH], bf16)
            y = jnp.dot(L, w, preferred_element_type=f32)
            store_tok(y.astype(bf16), c0, DH)
            yv[h] = jnp.concatenate([y[0:8], jnp.zeros((8, DH), f32)], axis=0).astype(bf16)

        def do_s(h):
            tok = rc[:, h * HW:h * HW + 2 * DH]
            a = jnp.concatenate([tok, yqk.pop(h)], axis=0)
            q = a[:, :DH]; k = a[:, DH:]
            s = lax.dot_general(q, k, _NT, preferred_element_type=f32)
            s = jnp.where(allowed, s, NEG)
            m = jnp.max(s, axis=1, keepdims=True)
            e = jnp.exp2(s - m)
            l = jnp.sum(e, axis=1, keepdims=True)
            r = pl.reciprocal(l, approx=True)
            r = r * (2.0 - l * r)
            es[h] = (e.astype(bf16), r)

        def do_v(h):
            p, r = es.pop(h)
            tok = rc[:, h * HW + 2 * DH:(h + 1) * HW]
            v = jnp.concatenate([tok, yv.pop(h)], axis=0)
            o = (jnp.dot(p, v, preferred_element_type=f32) * r).astype(bf16)
            oc[:, h * DH:(h + 1) * DH] = o[0:32]
            os_[h] = o[32:40]

        def do_o(h):
            lhs = jnp.concatenate([os_.pop(h)] + [ref[r0:r0 + n, h * DH:(h + 1) * DH] for (ref, r0, n) in op_pieces], axis=0)
            w = pltpu.bitcast(wop_ref[h * 128:(h + 1) * 128, :], bf16)
            y = jnp.dot(lhs, w, preferred_element_type=f32)
            acc[0] = y if acc[0] is None else acc[0] + y

        jobs = {"K": do_pqk, "P": do_pv, "S": do_s, "V": do_v, "O": do_o}
        for tok in ORDER:
            kind, idx = tok[0], tok[1:]
            if kind in jobs:
                jobs[kind](int(idx))
            else:
                for fn in fill.get(tok, ()):
                    fn()
        return acc[0]

    def superstep(j, mem, rOc, rOn, oOc, oOp, bta, btb, fills):
        xa = xb_ref[pl.ds(pl.multiple_of(j * 64 + 40, 8), 24), :]
        y2 = step(mem, xa, ringE, [(8, 24, rOc, 8)], oE, [(oOp, 0, 24)], fills[0])
        mem = y2[0:8].astype(bf16)
        for (r0, n, par, d0) in bta:
            bst_ref[par, d0:d0 + n, :] = y2[r0:r0 + n]
        nx = pl.multiple_of(jnp.minimum(j * 64 + 64, S - 40), 8)
        xn = xb_ref[pl.ds(nx, 40), :]
        y2 = step(mem, xn, rOc, [(8, 32, ringE, 0), (40, 8, rOn, 0)], oOc, [(oOp, 24, 8), (oE, 0, 32)], fills[1])
        mem = y2[0:8].astype(bf16)
        for (r0, n, par, d0) in btb:
            bst_ref[par, d0:d0 + n, :] = y2[r0:r0 + n]
        return mem

    def mkfill(pblk, pg, blk, g, opar, q):
        f = {}
        for hh in range(4):
            f["a%d" % hh] = [functools.partial(a_scores, blk, g, hh)]
            f["b%d" % hh] = [functools.partial(a_pv, blk, g, hh)]
            f["c%d" % hh] = [functools.partial(a_pv, pblk, pg, hh)]
        f["d0"] = [functools.partial(a_out, opar, 112 * q, 112)]
        if KLOOP:
            f["k0"] = [functools.partial(k_proj, jnp.minimum(blk + 1, NBLK - 1), g)]
        return f

    def body(i, mem):
        par = lax.rem(i, 2)
        prev = jnp.maximum(i - 1, 0)
        ppar = 1 - par

        @pl.when(i >= 3)
        def _():
            out_copy(i - 3).start()

        combine(par, i, jnp.maximum(i - 2, 0))
        f0 = mkfill(prev, 3, i, 0, ppar, 0)
        f1 = mkfill(i, 0, i, 1, ppar, 1)
        mem = superstep(2 * i, mem, ringOA, ringOB, oOA, oOB,
                        [(8, 24, ppar, 96)], [(8, 8, ppar, 120), (16, 32, par, 0)], (f0, f1))
        f2 = mkfill(i, 1, i, 2, ppar, 2)
        f3 = mkfill(i, 2, i, 3, ppar, 3)
        mem = superstep(2 * i + 1, mem, ringOB, ringOA, oOB, oOA,
                        [(8, 24, par, 32)], [(8, 40, par, 56)], (f2, f3))
        return mem

    niter = int(os.environ.get("NITER", NSUPER // 2))
    lax.fori_loop(0, niter, body, mem0_ref[...])

    nb = NBLK
    out_copy(nb - 3).start()
    w = pltpu.bitcast(wop_ref[...], bf16)
    y2 = jnp.dot(oOB[...], w, preferred_element_type=f32)
    for hh in (2, 3):
        a_pv(nb - 1, 3, hh)
    combine(0, nb, nb - 2)
    out_copy(nb - 2).start()
    a_out(1, 0, D)
    bst_ref[1, 96:128, :] = y2
    combine(1, nb + 1, nb - 1)
    out_copy(nb - 1).start()
    for b in list(range(max(niter - 3, 0))) + [nb - 3, nb - 2, nb - 1]:
        out_copy(b).wait()


@functools.partial(jax.jit, static_argnames=("B_seg_len",))
def pallas_gated_mix__sliding_block__memory_aug_recurrent_mem_tr__prompt_kernel(A_x, A_wqkv, A_wo, B_x, B_mem0, B_Wq, B_Wk, B_Wv, B_Wo, B_seg_len, gate_w):
    assert B_seg_len == SEG
    xaT = jnp.swapaxes(A_x, 1, 2).reshape(D, S)
    mem0 = B_mem0.reshape(M, D)
    wq = B_Wq.reshape(D * H, DH); wk = B_Wk.reshape(D * H, DH); wv = B_Wv.reshape(D * H, DH)
    woT = jnp.swapaxes(B_Wo, 1, 2).reshape(H * D, DH)
    outT = pl.pallas_call(
        _kernel,
        out_shape=jax.ShapeDtypeStruct((D, S), bf16),
        in_specs=[pl.BlockSpec(memory_space=pl.ANY)] * 9,
        out_specs=pl.BlockSpec(memory_space=pl.ANY),
        scratch_shapes=[
            pltpu.SemaphoreType.DMA((10,)),
            pltpu.VMEM((D, S), bf16),
            pltpu.VMEM((D, 3 * D), bf16),
            pltpu.VMEM((D, D), bf16),
            pltpu.VMEM((M, D), bf16),
            pltpu.VMEM((D,), bf16),
            pltpu.VMEM((D * H, DH), bf16), pltpu.VMEM((D * H, DH), bf16),
            pltpu.VMEM((D * H, DH), bf16), pltpu.VMEM((D * H, DH), bf16),
            pltpu.VMEM((14, 2, 128, 128), u32),
            pltpu.VMEM((224, NQKV), u32),
            pltpu.VMEM((H * 128, D), u32),
            pltpu.VMEM((S, D), bf16),
            pltpu.VMEM((SEG, NQKV), bf16), pltpu.VMEM((SEG, NQKV), bf16), pltpu.VMEM((SEG, NQKV), bf16),
            pltpu.VMEM((SEG, H * DH), bf16), pltpu.VMEM((SEG, H * DH), bf16), pltpu.VMEM((SEG, H * DH), bf16),
            pltpu.VMEM((2, 128, D), f32),
            pltpu.VMEM((2 * AN + 16, D), bf16),
            pltpu.VMEM((D, AN), bf16),
            pltpu.VMEM((4, D // 2, 128), u32),
            pltpu.VMEM((AN, S), bf16),
            pltpu.VMEM((4, (AW + S) // 2, 128), u32),
            pltpu.VMEM((AN, AW + S), bf16),
            pltpu.VMEM((8, S), f32),
            pltpu.VMEM((4, 384, 128), bf16),
            pltpu.VMEM((2, AN // 2, 128), u32),
            pltpu.VMEM((D, S + 256), bf16),
            pltpu.VMEM((2, D, 128), f32),
            pltpu.VMEM((4, 128, 256), bf16),
            pltpu.VMEM((4, 256, 128), bf16),
        ],
        compiler_params=pltpu.CompilerParams(vmem_limit_bytes=120 * 1024 * 1024),
    )(xaT, A_wqkv, A_wo, mem0, wq, wk, wv, woT, gate_w)
    return jnp.swapaxes(outT.reshape(1, D, S), 1, 2)
```

```python
import functools
import jax
import jax.numpy as jnp
from jax import lax
from jax.experimental import pallas as pl
from jax.experimental.pallas import tpu as pltpu

bf16, f32, u32 = jnp.bfloat16, jnp.float32, jnp.uint32

S, D = 2048, 448
ADH, AW = 28, 256
APD = 32
AN = 16 * APD
H, DH, M, SEG = 16, 256, 8, 32
HW = 3 * DH
NQKV = H * HW
LOG2E = 1.4426950408889634
B_QSCALE = (DH ** -0.5) * LOG2E
A_QSCALE = (ADH ** -0.5) * LOG2E
NEG = -1e30
MASKVAL = -1e9
NSUPER = S // (2 * SEG)
NBLK = S // 128
CH = 256


KA, LV, LO = 4, 2, 6


def _order(extra, tail):
    tl = tail.split()
    o = ["K%d" % i for i in range(KA)]
    done = set()
    for t in range(16):
        if t + KA < 16: o.append("K%d" % (t + KA))
        for p in range(8):
            if "S%d" % p not in done and 2 * p + 1 <= min(t + KA - 1, 15):
                o.append("S%d" % p); done.add("S%d" % p)
        o.append("P%d" % t)
        o += extra.get(t, [])
        if (t - LV) % 2 == 1 and t >= LV: o.append("V%d" % ((t - LV) // 2)); done.add(o[-1])
        if t >= LO: o.append("O%d" % (t - LO)); done.add(o[-1])
    rest = ["V%d" % p for p in range(8) if "V%d" % p not in done] + ["O%d" % h for h in range(16) if "O%d" % h not in done]
    assert all(r in tl for r in rest), (rest, tl)
    return o + tl


def _parse_extra(s):
    d = {}
    for item in s.split():
        slot, job = item.split(":")
        d.setdefault(int(slot), []).append(job)
    return d


_TAIL = "O10 a0 O11 V7 O12 a1 O13 a2 O14 a3 O15 d0"
_EX = "0:c0 1:c1 2:c2 3:c3"
ORDERS = [_order(_parse_extra(_EX), _TAIL)] * 4

_NT = (((1,), (1,)), ((), ()))


def _perm_t(off, wl):
    n = lax.broadcasted_iota(jnp.int32, (128, wl), 0)
    s = lax.broadcasted_iota(jnp.int32, (128, wl), 1)
    hit = (s == off + ADH * (n >> 5) + (n & 31)) & ((n & 31) < ADH)
    return jnp.where(hit, 1.0, 0.0).astype(bf16)


def _perm(off, wl):
    s = lax.broadcasted_iota(jnp.int32, (wl, 128), 0)
    n = lax.broadcasted_iota(jnp.int32, (wl, 128), 1)
    hit = (s == off + ADH * (n >> 5) + (n & 31)) & ((n & 31) < ADH)
    return jnp.where(hit, 1.0, 0.0).astype(bf16)


def _kernel(xaT_hbm, wqkv_hbm, woa_hbm, mem0_hbm, wq_hbm, wk_hbm, wv_hbm, woT_hbm, gate_hbm,
            out_hbm,
            sems, xaT_ref, wqkv_ref, woa_ref, mem0_ref, gate_ref, wr0, wr1, wr2, wr3,
            t_ref, wp_ref, wop_ref, xb_ref, ringE, ringOA, ringOB, oE, oOA, oOB, bst_ref,
            wT_ref, wkp_ref, woTp_ref, qT_ref, kA_ref, vT_ref, g_ref, pT_ref, oT_ref, outT_ref, aT_ref,
            pmt_ref, pmk_ref):
    def cp(src, dst, k):
        return pltpu.make_async_copy(src, dst, sems.at[k])

    c_w0 = cp(wqkv_hbm.at[:, 0:512], wqkv_ref.at[:, 0:512], 0)
    c_w1 = cp(wqkv_hbm.at[:, 512:896], wqkv_ref.at[:, 512:896], 10)
    c_w2 = cp(wqkv_hbm.at[:, 896:3 * D], wqkv_ref.at[:, 896:3 * D], 11)
    c_xa0 = cp(xaT_hbm.at[:, 0:CH], xaT_ref.at[:, 0:CH], 1)
    c_xa1 = cp(xaT_hbm.at[:, CH:S], xaT_ref.at[:, CH:S], 12)
    c_woa = cp(woa_hbm, woa_ref, 2)
    c_gate, c_mem0 = cp(gate_hbm, gate_ref, 3), cp(mem0_hbm, mem0_ref, 4)
    c_wq, c_wk, c_wo = cp(wq_hbm, wr0, 5), cp(wk_hbm, wr1, 6), cp(woT_hbm, wr3, 8)
    HV = D * H // 2
    c_wv0 = cp(wv_hbm.at[0:HV, :], wr2.at[0:HV, :], 7)
    c_wv1 = cp(wv_hbm.at[HV:2 * HV, :], wr2.at[HV:2 * HV, :], 13)
    for c in (c_w0, c_gate, c_w2, c_w1, c_xa0, c_xa1, c_mem0, c_woa, c_wq, c_wo, c_wk, c_wv0, c_wv1):
        c.start()

    qwin = [(112 * g // 128) * 128 for g in range(4)]
    kwin = [((D + 112 * g) // 128) * 128 for g in range(4)]
    qwl = [128, 256, 256, 192]
    kwl = [256, 256, 256, 128]
    for g in range(4):
        pmt_ref[g] = _perm_t(112 * g - qwin[g], 256)
        pmk_ref[g] = _perm(D + 112 * g - kwin[g], 256)
    lane = lax.broadcasted_iota(jnp.int32, (AW // 2, 128), 1)
    for g in range(4):
        kA_ref[g, 0:AW // 2, :] = jnp.where((lane & 31) == ADH, u32(0x3F803F80), u32(0))
    vT_ref[:, 0:AW] = jnp.zeros((AN, AW), bf16)
    pT_ref[...] = jnp.ones(pT_ref.shape, bf16)
    aT_ref[...] = jnp.zeros(aT_ref.shape, f32)
    oT_ref[...] = jnp.zeros(oT_ref.shape, u32)
    bst_ref[...] = jnp.zeros(bst_ref.shape, f32)
    oOB[...] = jnp.zeros(oOB.shape, bf16)

    for cw, base, row0 in ((c_w0, 0, 0), (c_w2, 2 * D, AN)):
        cw.wait()
        for g in range(4):
            w0, wl = base + qwin[g], qwl[g]
            y = lax.dot_general(pmt_ref[g, :, 0:wl], wqkv_ref[:, w0:w0 + wl], _NT, preferred_element_type=f32)
            wT_ref[row0 + 128 * g: row0 + 128 * (g + 1), :] = y.astype(bf16)
    c_w1.wait()
    for g in range(4):
        w0, wl = kwin[g], kwl[g]
        y = jnp.dot(wqkv_ref[:, w0:w0 + wl], pmk_ref[g, 0:wl, :], preferred_element_type=f32)
        wkp_ref[:, 128 * g:128 * (g + 1)] = y.astype(bf16)
    c_gate.wait()
    wT_ref[2 * AN:2 * AN + 16, :] = jnp.broadcast_to(gate_ref[...].reshape(1, D), (16, D))
    c_xa0.wait()

    def relayout_unit(w_ref, part, g, slot):
        r0 = pl.multiple_of(g * 256, 256)
        o0 = pl.multiple_of(g * 8, 8)
        for c in range(2):
            t = pltpu.bitcast(w_ref[pl.ds(r0, 256), c * 128:(c + 1) * 128], u32)
            for dd in range(16):
                p0 = (dd % 2) * 64 + (dd // 2) * 8
                t_ref[slot, c, p0:p0 + 8, :] = t[dd * 8:(dd + 1) * 8]
        for c in range(2):
            for i in range(8):
                a = t_ref[slot, c, pl.ds(i, 8, stride=8), :]
                b = t_ref[slot, c, pl.ds(64 + i, 8, stride=8), :]
                x = (a & u32(0xFFFF)) | (b << 16)
                y = (a >> 16) | (b & u32(0xFFFF0000))
                ca = (2 * i) * HW + part * DH + c * 128
                cb = (2 * i + 1) * HW + part * DH + c * 128
                wp_ref[pl.ds(o0, 8), ca:ca + 128] = x
                wp_ref[pl.ds(o0, 8), cb:cb + 128] = y

    def aproj(c, extra):
        extra = list(extra)
        per = -(-len(extra) // 5)

        def run_extra():
            for _ in range(per):
                if extra:
                    extra.pop(0)()

        c0 = pl.multiple_of(c * CH, CH)
        xT = xaT_ref[:, pl.ds(c0, CH)]
        row = lax.broadcasted_iota(jnp.int32, (256, CH), 0)
        for p in range(2):
            y = jnp.dot(wT_ref[256 * p:256 * (p + 1), :], xT, preferred_element_type=f32)
            q = jnp.where((row & 31) == ADH, MASKVAL, y * A_QSCALE)
            qT_ref[256 * p:256 * (p + 1), pl.ds(c0, CH)] = q.astype(bf16)
            run_extra()
        y = jnp.dot(wT_ref[AN:AN + 256, :], xT, preferred_element_type=f32)
        vT_ref[0:256, pl.ds(AW + c0, CH)] = jnp.where((row & 31) == ADH, 1.0, y).astype(bf16)
        run_extra()
        y = jnp.dot(wT_ref[AN + 256:2 * AN + 16, :], xT, preferred_element_type=f32)
        vT_ref[256:512, pl.ds(AW + c0, CH)] = jnp.where((row & 31) == ADH, 1.0, y[0:256]).astype(bf16)
        g_ref[:, pl.ds(c0, CH)] = jax.nn.sigmoid(y[256:264])
        run_extra()
        xr = xT.T
        kk = jnp.dot(xr, wkp_ref[...], preferred_element_type=f32).astype(bf16)
        for g in range(4):
            kA_ref[g, pl.ds(pl.multiple_of((AW + c0) // 2, 64), CH // 2), :] = pltpu.bitcast(kk[:, 128 * g:128 * (g + 1)], u32)
        xb_ref[pl.ds(c0, CH), :] = xr
        run_extra()

    def wo_unit(h):
        r0 = pl.multiple_of(h * D, 64)
        q0 = pl.multiple_of(h * 128, 128)
        wop_ref[pl.ds(q0, 128), :] = pltpu.bitcast(wr3[pl.ds(r0, D), :].T, u32)

    def aproj_relay(c, _, w_ref, part, c_first, n):
        aproj(c_first + c, [functools.partial(relayout_unit, w_ref, part, c * n + u, u % 14) for u in range(n)])
        return 0

    def aproj_wo(c, _):
        aproj(5 + c, [functools.partial(wo_unit, c * 8 + u) for u in range(8)])
        return 0

    aproj(0, [])
    c_xa1.wait()
    for c in range(1, 4):
        aproj(c, [])
    c_wq.wait()
    aproj_relay(0, 0, wr0, 0, 4, 28)
    c_wo.wait()
    for c in range(2):
        aproj_wo(c, 0)
    c_wk.wait()
    aproj_relay(0, 0, wr1, 1, 7, 28)

    c_woa.wait()
    c_mem0.wait()
    L0 = xb_ref[0:48, :]

    def wo_a(c):
        w0 = min((112 * c // 128) * 128, D - 256)
        n = lax.broadcasted_iota(jnp.int32, (128, 256), 0)
        s = lax.broadcasted_iota(jnp.int32, (128, 256), 1)
        hit = (s == 112 * c - w0 + ADH * (n >> 5) + (n & 31)) & ((n & 31) < ADH)
        y = jnp.dot(jnp.where(hit, 1.0, 0.0).astype(bf16), woa_ref[w0:w0 + 256, :], preferred_element_type=f32)
        woTp_ref[c] = pltpu.bitcast(y.T.astype(bf16), u32)

    def pro_qk(h):
        c0 = h * HW
        w = pltpu.bitcast(wp_ref[:, pl.ds(c0, 2 * DH)], bf16)
        y = jnp.dot(L0, w, preferred_element_type=f32)
        y = jnp.concatenate([y[:, :DH] * B_QSCALE, y[:, DH:]], axis=1)
        yb = y.astype(bf16)
        ringE[:, pl.ds(c0, 2 * DH)] = yb[0:32]
        ringOA[0:8, pl.ds(c0, 2 * DH)] = yb[32:40]

    for h in range(8):
        pro_qk(h)
    c_wv0.wait()
    for h in range(8, 12):
        pro_qk(h)
        for u in range(4 * (h - 8), min(4 * (h - 8) + 4, 14)):
            relayout_unit(wr2, 2, u, u % 14)
    c_wv1.wait()
    for h in range(12, 16):
        pro_qk(h)
        for u in range(14 + 4 * (h - 12), min(14 + 4 * (h - 12) + 4, 28)):
            relayout_unit(wr2, 2, u, u % 14)
    for h in range(H):
        c0 = h * HW + 2 * DH
        w = pltpu.bitcast(wp_ref[:, c0:c0 + DH], bf16)
        yb = jnp.dot(L0, w, preferred_element_type=f32).astype(bf16)
        ringE[:, c0:c0 + DH] = yb[0:32]
        ringOA[0:8, c0:c0 + DH] = yb[32:40]
        if h % 4 == 0:
            wo_a(h // 4)

    ri = lax.broadcasted_iota(jnp.int32, (80, 96), 0)
    ci = lax.broadcasted_iota(jnp.int32, (80, 96), 1)
    row_h1 = ((ri >= 32) & (ri < 64)) | (ri >= 72)
    col_h1 = ci >= 48
    kj = jnp.where(col_h1, ci - 48, ci)
    allowed = (row_h1 == col_h1) & (kj < 40) & ((ri >= 64) | (kj >= 32) | (kj <= (ri & 31)))
    tri = lax.broadcasted_iota(jnp.int32, (128, 128), 0) <= lax.broadcasted_iota(jnp.int32, (128, 128), 1)

    def a_scores(blk, g, hh):
        b0 = pl.multiple_of(blk * 128, 128)
        h = 4 * g + hh
        parts = []
        if hh > 0:
            parts.append(jnp.zeros((32 * hh, 128), bf16))
        parts.append(qT_ref[32 * h:32 * (h + 1), pl.ds(b0, 128)])
        if hh < 3:
            parts.append(jnp.zeros((96 - 32 * hh, 128), bf16))
        w = jnp.concatenate(parts, axis=0)
        kr = pltpu.bitcast(kA_ref[g, pl.ds(pl.multiple_of(blk * 64, 64), 192), :], bf16)
        s = jnp.dot(kr, w, preferred_element_type=f32)
        sm = jnp.where(tri, s[256:384], s[0:128])
        s2 = s[128:256]
        m = jnp.max(jnp.maximum(sm, s2), axis=0, keepdims=True)
        em = jnp.exp2(sm - m)
        e2 = jnp.exp2(s2 - m)
        pT_ref[hh, 0:128, :] = jnp.where(tri, 0.0, em).astype(bf16)
        pT_ref[hh, 128:256, :] = e2.astype(bf16)
        pT_ref[hh, 256:384, :] = jnp.where(tri, em, 0.0).astype(bf16)

    def a_pv(blk, bpar, g, hh):
        b0 = pl.multiple_of(blk * 128, 128)
        h = 4 * g + hh
        v = vT_ref[32 * h:32 * (h + 1), pl.ds(b0, 384)]
        o = jnp.dot(v, pT_ref[hh], preferred_element_type=f32)
        l = o[ADH:ADH + 1, :]
        r = pl.reciprocal(l, approx=True)
        r = r * (2.0 - l * r)
        o = o * r
        oT_ref[bpar, 16 * h:16 * (h + 1), :] = pltpu.bitcast(o.astype(bf16), u32)

    def a_out(par, r0, n):
        lhs = pltpu.bitcast(jnp.concatenate([woTp_ref[g, r0 // 2:(r0 + n) // 2, :] for g in range(4)], axis=1), bf16)
        aT_ref[par, r0:r0 + n, :] = jnp.dot(lhs, pltpu.bitcast(oT_ref[par], bf16), preferred_element_type=f32)

    def combine(par, slot, gblk):
        c0 = pl.multiple_of(slot * 128, 128)
        gb = pl.multiple_of(gblk * 128, 128)
        g = g_ref[0:1, pl.ds(gb, 128)]
        bT = bst_ref[par].T
        outT_ref[:, pl.ds(c0, 128)] = (g * aT_ref[par] + (1.0 - g) * bT).astype(bf16)

    def out_copy(blk):
        c0 = pl.multiple_of(blk * 128, 128)
        return pltpu.make_async_copy(outT_ref.at[:, pl.ds(256 + c0, 128)], out_hbm.at[:, pl.ds(c0, 128)], sems.at[9])

    def step(mem, xrows, rc, n_targets, oc, op_pieces, fill, order):
        L = jnp.concatenate([mem, xrows], axis=0)
        yqk, yv, es, os_ = {}, {}, {}, {}
        acc = [None]

        def store_tok(yb, c0, w):
            for (r0, n, ref, d0) in n_targets:
                ref[d0:d0 + n, c0:c0 + w] = yb[r0:r0 + n]

        def do_pqk(h):
            c0 = h * HW
            w = pltpu.bitcast(wp_ref[:, c0:c0 + 2 * DH], bf16)
            y = jnp.dot(L, w, preferred_element_type=f32)
            y = jnp.concatenate([y[:, :DH] * B_QSCALE, y[:, DH:]], axis=1)
            store_tok(y.astype(bf16), c0, 2 * DH)
            yqk[h] = y[0:8]

        def do_pv(h):
            c0 = h * HW + 2 * DH
            w = pltpu.bitcast(wp_ref[:, c0:c0 + DH], bf16)
            y = jnp.dot(L, w, preferred_element_type=f32)
            store_tok(y.astype(bf16), c0, DH)
            yv[h] = jnp.concatenate([y[0:8], jnp.zeros((8, DH), f32)], axis=0).astype(bf16)

        def do_s(p):
            h0, h1 = 2 * p, 2 * p + 1
            t0 = rc[:, h0 * HW:h0 * HW + 2 * DH]
            t1 = rc[:, h1 * HW:h1 * HW + 2 * DH]
            m0, m1 = yqk.pop(h0), yqk.pop(h1)
            qm = jnp.concatenate([m0[:, :DH], m1[:, :DH]], axis=0).astype(bf16)
            q = jnp.concatenate([t0[:, :DH], t1[:, :DH], qm], axis=0)
            zk = jnp.zeros((8, DH), f32)
            k = jnp.concatenate([t0[:, DH:], jnp.concatenate([m0[:, DH:], zk], axis=0).astype(bf16),
                                 t1[:, DH:], jnp.concatenate([m1[:, DH:], zk], axis=0).astype(bf16)], axis=0)
            s = lax.dot_general(q, k, _NT, preferred_element_type=f32)
            s = jnp.where(allowed, s, NEG)
            m = jnp.max(s, axis=1, keepdims=True)
            e = jnp.exp2(s - m)
            l = jnp.sum(e, axis=1, keepdims=True)
            r = pl.reciprocal(l, approx=True)
            r = r * (2.0 - l * r)
            es[p] = (e * r).astype(bf16)

        def do_v(p):
            h0, h1 = 2 * p, 2 * p + 1
            v = jnp.concatenate([rc[:, h0 * HW + 2 * DH:(h0 + 1) * HW], yv.pop(h0),
                                 rc[:, h1 * HW + 2 * DH:(h1 + 1) * HW], yv.pop(h1)], axis=0)
            o = jnp.dot(es.pop(p), v, preferred_element_type=f32).astype(bf16)
            oc[:, h0 * DH:(h0 + 1) * DH] = o[0:32]
            oc[:, h1 * DH:(h1 + 1) * DH] = o[32:64]
            os_[h0] = o[64:72]
            os_[h1] = o[72:80]

        def do_o(h):
            lhs = jnp.concatenate([os_.pop(h)] + [ref[r0:r0 + n, h * DH:(h + 1) * DH] for (ref, r0, n) in op_pieces], axis=0)
            w = pltpu.bitcast(wop_ref[h * 128:(h + 1) * 128, :], bf16)
            y = jnp.dot(lhs, w, preferred_element_type=f32)
            acc[0] = y if acc[0] is None else acc[0] + y

        jobs = {"K": do_pqk, "P": do_pv, "S": do_s, "V": do_v, "O": do_o}
        for tok in order:
            kind, idx = tok[0], tok[1:]
            if kind in jobs:
                jobs[kind](int(idx))
            else:
                for fn in fill.get(tok, ()):
                    fn()
        return acc[0]

    def superstep(j, mem, rOc, rOn, oOc, oOp, bta, btb, fills, orders):
        xa = xb_ref[pl.ds(pl.multiple_of(j * 64 + 40, 8), 24), :]
        y2 = step(mem, xa, ringE, [(8, 24, rOc, 8)], oE, [(oOp, 0, 24)], fills[0], orders[0])
        mem = y2[0:8].astype(bf16)
        for (r0, n, par, d0) in bta:
            bst_ref[par, d0:d0 + n, :] = y2[r0:r0 + n]
        nx = pl.multiple_of(jnp.minimum(j * 64 + 64, S - 40), 8)
        xn = xb_ref[pl.ds(nx, 40), :]
        y2 = step(mem, xn, rOc, [(8, 32, ringE, 0), (40, 8, rOn, 0)], oOc, [(oOp, 24, 8), (oE, 0, 32)], fills[1], orders[1])
        mem = y2[0:8].astype(bf16)
        for (r0, n, par, d0) in btb:
            bst_ref[par, d0:d0 + n, :] = y2[r0:r0 + n]
        return mem

    def mkfill(pblk, ppar_, pg, blk, par_, g, opar, q):
        f = {}
        for hh in range(4):
            f["a%d" % hh] = [functools.partial(a_scores, blk, g, hh)]
            f["b%d" % hh] = [functools.partial(a_pv, blk, par_, g, hh)]
            f["c%d" % hh] = [functools.partial(a_pv, pblk, ppar_, pg, hh)]
        f["d0"] = [functools.partial(a_out, opar, 112 * q, 112)]
        return f

    def body(i, mem):
        par = lax.rem(i, 2)
        prev = jnp.maximum(i - 1, 0)
        ppar = 1 - par

        @pl.when(i >= 3)
        def _():
            out_copy(i - 3).start()

        combine(par, i, jnp.maximum(i - 2, 0))
        f0 = mkfill(prev, ppar, 3, i, par, 0, ppar, 0)
        f1 = mkfill(i, par, 0, i, par, 1, ppar, 1)
        mem = superstep(2 * i, mem, ringOA, ringOB, oOA, oOB,
                        [(8, 24, ppar, 96)], [(8, 8, ppar, 120), (16, 32, par, 0)], (f0, f1), ORDERS[0:2])
        f2 = mkfill(i, par, 1, i, par, 2, ppar, 2)
        f3 = mkfill(i, par, 2, i, par, 3, ppar, 3)
        mem = superstep(2 * i + 1, mem, ringOB, ringOA, oOB, oOA,
                        [(8, 24, par, 32)], [(8, 40, par, 56)], (f2, f3), ORDERS[2:4])
        return mem

    niter = NSUPER // 2
    lax.fori_loop(0, niter, body, mem0_ref[...])

    nb = NBLK
    out_copy(nb - 3).start()
    w = pltpu.bitcast(wop_ref[...], bf16)
    y2 = jnp.dot(oOB[...], w, preferred_element_type=f32)
    for hh in range(4):
        if "b%d" % hh not in ORDERS[3]:
            a_pv(nb - 1, 1, 3, hh)
    combine(0, nb, nb - 2)
    out_copy(nb - 2).start()
    a_out(1, 0, D)
    bst_ref[1, 96:128, :] = y2
    combine(1, nb + 1, nb - 1)
    out_copy(nb - 1).start()
    for b in list(range(max(niter - 3, 0))) + [nb - 3, nb - 2, nb - 1]:
        out_copy(b).wait()


@functools.partial(jax.jit, static_argnames=("B_seg_len",))
def pallas_gated_mix__sliding_block__memory_aug_recurrent_mem_tr__prompt_kernel(A_x, A_wqkv, A_wo, B_x, B_mem0, B_Wq, B_Wk, B_Wv, B_Wo, B_seg_len, gate_w):
    assert B_seg_len == SEG
    xaT = jnp.swapaxes(A_x, 1, 2).reshape(D, S)
    mem0 = B_mem0.reshape(M, D)
    wq = B_Wq.reshape(D * H, DH); wk = B_Wk.reshape(D * H, DH); wv = B_Wv.reshape(D * H, DH)
    woT = jnp.swapaxes(B_Wo, 1, 2).reshape(H * D, DH)
    outT = pl.pallas_call(
        _kernel,
        out_shape=jax.ShapeDtypeStruct((D, S), bf16),
        in_specs=[pl.BlockSpec(memory_space=pl.ANY)] * 9,
        out_specs=pl.BlockSpec(memory_space=pl.ANY),
        scratch_shapes=[
            pltpu.SemaphoreType.DMA((14,)),
            pltpu.VMEM((D, S), bf16),
            pltpu.VMEM((D, 3 * D), bf16),
            pltpu.VMEM((D, D), bf16),
            pltpu.VMEM((M, D), bf16),
            pltpu.VMEM((D,), bf16),
            pltpu.VMEM((D * H, DH), bf16), pltpu.VMEM((D * H, DH), bf16),
            pltpu.VMEM((D * H, DH), bf16), pltpu.VMEM((D * H, DH), bf16),
            pltpu.VMEM((14, 2, 128, 128), u32),
            pltpu.VMEM((224, NQKV), u32),
            pltpu.VMEM((H * 128, D), u32),
            pltpu.VMEM((S, D), bf16),
            pltpu.VMEM((SEG, NQKV), bf16), pltpu.VMEM((SEG, NQKV), bf16), pltpu.VMEM((SEG, NQKV), bf16),
            pltpu.VMEM((SEG, H * DH), bf16), pltpu.VMEM((SEG, H * DH), bf16), pltpu.VMEM((SEG, H * DH), bf16),
            pltpu.VMEM((2, 128, D), f32),
            pltpu.VMEM((2 * AN + 16, D), bf16),
            pltpu.VMEM((D, AN), bf16),
            pltpu.VMEM((4, D // 2, 128), u32),
            pltpu.VMEM((AN, S), bf16),
            pltpu.VMEM((4, (AW + S) // 2, 128), u32),
            pltpu.VMEM((AN, AW + S), bf16),
            pltpu.VMEM((8, S), f32),
            pltpu.VMEM((4, 384, 128), bf16),
            pltpu.VMEM((2, AN // 2, 128), u32),
            pltpu.VMEM((D, S + 256), bf16),
            pltpu.VMEM((2, D, 128), f32),
            pltpu.VMEM((4, 128, 256), bf16),
            pltpu.VMEM((4, 256, 128), bf16),
        ],
        compiler_params=pltpu.CompilerParams(vmem_limit_bytes=120 * 1024 * 1024),
    )(xaT, A_wqkv, A_wo, mem0, wq, wk, wv, woT, gate_w)
    return jnp.swapaxes(outT.reshape(1, D, S), 1, 2)
```
